```python
import os as _os
_os.environ.setdefault("JAX_PLATFORMS", "cpu")
import jax
import jax.numpy as jnp

def _softmax(x, axis=-1):
    return jax.nn.softmax(x, axis=axis)
def _gelu(x):
    return jax.nn.gelu(x, approximate=True)
def _silu(x):
    return jax.nn.silu(x)
def _sigmoid(x):
    return jax.nn.sigmoid(x)
def _layernorm(x, axis=-1, eps=1e-5):
    m = jnp.mean(x, axis=axis, keepdims=True)
    v = jnp.var(x, axis=axis, keepdims=True)
    return (x - m) / jnp.sqrt(v + eps)
def _scatter_add(tgt, idx, src, axis=0):
    return tgt.at[idx].add(src)
def _segment_sum(src, seg, n):
    return jax.ops.segment_sum(src, seg, n)
class _Rng:
    def __init__(self, key):
        self._k = key
    def _next(self):
        self._k, sub = jax.random.split(self._k)
        return sub
    def normal(self, shape):
        return jax.random.normal(self._next(), shape, dtype=jnp.bfloat16)
    def randint(self, lo, hi, shape):
        return jax.random.randint(self._next(), shape, lo, hi, dtype=jnp.int32)
    def uniform(self, shape, lo=0.0, hi=1.0):
        return jax.random.uniform(self._next(), shape, jnp.bfloat16, lo, hi)
    def permutation(self, n):
        return jax.random.permutation(self._next(), n)


kernel_name = 'standalone__linear_kernel_rfa__decode'

def setup_inputs():
    _rng = _Rng(jax.random.key(int.from_bytes(__import__("os").urandom(4), "little")))
    _w = (lambda a: (lambda t: t.astype(jnp.bfloat16) if jnp.issubdtype(t.dtype, jnp.floating) else t)(jnp.asarray(a)))
    B, H, Sq, Sk, D, M = 2, 16, 1, 16384, 256, 16
    return {
        "q": _w((lambda *s: _rng.normal(s) * 0.4)(B, H, Sq, D)),
        "k": _w((lambda *s: _rng.normal(s) * 1.6)(B, H, Sk, D)),
        "v": _w((lambda *s: _rng.normal(s) * 1.6)(B, H, Sk, D)),
        "omega": _w((lambda *s: _rng.normal(s) * 1.6)(M, D)),
    }

def reference(q, k, v, omega):
    d = q.shape[-1]
    m = omega.shape[0]
    scale = float(d) ** -0.25
    qs = q * scale
    ks = k * scale
    q_proj = jnp.einsum("bhsd,md->bhsm", qs, omega)
    k_proj = jnp.einsum("bhsd,md->bhsm", ks, omega)
    q_sq = 0.5 * jnp.einsum("bhsd,bhsd->bhs", qs, qs)[..., None]
    k_sq = 0.5 * jnp.einsum("bhsd,bhsd->bhs", ks, ks)[..., None]
    inv_sqrt_m = float(m) ** -0.5
    phi_q = jnp.exp(q_proj - q_sq) * inv_sqrt_m + 1e-6
    phi_k = jnp.exp(k_proj - k_sq) * inv_sqrt_m + 1e-6
    kv = jnp.einsum("bhsm,bhsd->bhmd", phi_k, v)
    z  = jnp.einsum("bhsm->bhm", phi_k)
    num = jnp.einsum("bhqm,bhmd->bhqd", phi_q, kv)
    den = jnp.einsum("bhqm,bhm->bhq", phi_q, z)[..., None] + 1e-6
    return num / den
```

```python
import jax
import jax.numpy as jnp
from jax import lax
import jax.experimental.pallas as pl
import jax.experimental.pallas.tpu as pltpu

_NT = (((1,), (1,)), ((), ()))
_NN = (((1,), (0,)), ((), ()))

_R = 2048
_NB = 4
_RS = 64
_PIECES = (1024, 512, 256, 128, 128)


def _kernel(q_hbm, k_hbm, v_hbm, om_hbm, o_ref,
            kbuf, vbuf, qbuf, ombuf, ksem, vsem, auxsem, tailsem,
            phiq_ref, acc_ref, den_ref, out_ref):
    R, NB, r, pieces = _R, _NB, _RS, _PIECES
    NBK, NBV = NB, NB - 1
    nsub = R // r
    P = len(pieces)
    offs = [sum(pieces[:p]) for p in range(P)]

    BH, D = q_hbm.shape
    M = om_hbm.shape[0]
    S = k_hbm.shape[0] // BH
    CPH = S // R
    N = BH * CPH
    scale = float(D) ** -0.25
    inv_sqrt_m = float(M) ** -0.5
    f32 = jnp.float32
    bf16 = jnp.bfloat16

    def k_sub(c, off, prio):
        slot = c % NBK
        pltpu.make_async_copy(k_hbm.at[pl.ds(c * R + off, r)],
                              kbuf.at[slot, pl.ds(off, r)],
                              ksem.at[slot]).start(priority=prio)

    def v_sub(c, off, prio, sem=None):
        slot = c % NBV
        pltpu.make_async_copy(v_hbm.at[pl.ds(c * R + off, r)],
                              vbuf.at[slot, pl.ds(off, r)],
                              vsem.at[slot] if sem is None else sem
                              ).start(priority=prio)

    def issue_first():
        def f(s, _):
            off = pl.multiple_of(s * (2 * r), 2 * r)
            k_sub(0, off, 0)
            k_sub(0, off + r, 1)
            return 0
        lax.fori_loop(0, nsub // 2, f, 0)

    def issue_step(t):
        def f(s, _):
            off = pl.multiple_of(s * r, r)
            k_sub(t, off, 0)
            v_sub(t - 1, off, 1)
            return 0
        lax.fori_loop(0, nsub, f, 0)

    def issue_last():
        def f(s, _):
            off = pl.multiple_of(s * (2 * r), 2 * r)
            idx = 0
            for p in range(1, P):
                idx = idx + (off >= offs[p]).astype(jnp.int32)
            v_sub(N - 1, off, 0, tailsem.at[idx])
            v_sub(N - 1, off + r, 1, tailsem.at[idx])
            return 0
        lax.fori_loop(0, nsub // 2, f, 0)

    def k_wait(c):
        slot = c % NBK
        pltpu.make_async_copy(kbuf.at[slot], kbuf.at[slot], ksem.at[slot]).wait()

    def v_wait(c):
        slot = c % NBV
        pltpu.make_async_copy(vbuf.at[slot], vbuf.at[slot], vsem.at[slot]).wait()

    q_cp = pltpu.make_async_copy(q_hbm, qbuf, auxsem.at[0])
    om_cp = pltpu.make_async_copy(om_hbm, ombuf, auxsem.at[1])
    q_cp.start()
    om_cp.start()
    issue_first()
    for t in range(1, NB):
        issue_step(t)
    q_cp.wait()
    om_cp.wait()

    om = ombuf[...]
    omf = om.astype(f32)
    qs_all = qbuf[...].astype(f32) * scale
    for h in range(BH):
        qs = qs_all[h:h + 1, :]
        t = omf * qs - 0.5 * (qs * qs)
        e = jnp.sum(t, axis=1, keepdims=True)
        phi_q = jnp.exp(e) * inv_sqrt_m + 1e-6
        phiq_ref[h] = jnp.broadcast_to(phi_q, (M, 128))
    ones = jnp.ones((M, D // 2), bf16)

    def k_side(k, phiq):
        n = k.shape[0]
        pt = lax.dot_general(om, k, _NT, preferred_element_type=f32)
        kf = k.astype(f32)
        sq = kf * kf
        sqp = (sq[:, :D // 2] + sq[:, D // 2:]).astype(bf16)
        kst = lax.dot_general(ones, sqp, _NT, preferred_element_type=f32)
        e = pt * scale - kst * (0.5 * scale * scale)
        phi = jnp.exp(e) * inv_sqrt_m + 1e-6
        pw = phi * jnp.tile(phiq, (1, n // 128))
        w8 = pw[:8] + pw[8:]
        hi = w8.astype(bf16)
        lo = (w8 - hi.astype(f32)).astype(bf16)
        lhs = jnp.concatenate([hi, lo], axis=0)
        den = w8[:, 0:128]
        for t in range(1, n // 128):
            den = den + w8[:, t * 128:(t + 1) * 128]
        return lhs, den

    def total(den):
        return jnp.sum(jnp.sum(den, axis=0, keepdims=True), axis=1, keepdims=True) + 1e-6

    def body(c, carry):
        h = c // CPH
        j = c % CPH

        @pl.when(j == 0)
        def _():
            acc_ref[...] = jnp.zeros_like(acc_ref)
            den_ref[...] = jnp.zeros_like(den_ref)

        phiq = phiq_ref[h]
        k_wait(c)
        v_wait(c)
        lhs, dd = k_side(kbuf[c % NBK], phiq)
        acc = acc_ref[...] + lax.dot_general(lhs, vbuf[c % NBV], _NN,
                                             preferred_element_type=f32)
        den = den_ref[...] + dd
        acc_ref[...] = acc
        den_ref[...] = den

        @pl.when(c + NB < N)
        def _():
            issue_step(c + NB)

        @pl.when(c + NB == N)
        def _():
            issue_last()

        @pl.when(j == CPH - 1)
        def _():
            out_ref[pl.ds(h, 1), :] = jnp.sum(acc, axis=0, keepdims=True) / total(den)

        return carry

    lax.fori_loop(0, N - 1, body, 0)

    ks = (N - 1) % NBK
    vs = (N - 1) % NBV
    k_wait(N - 1)
    acc = acc_ref[...]
    lhs, dd = k_side(kbuf[ks], phiq_ref[BH - 1])
    d = total(den_ref[...] + dd)
    for p in range(P):
        dst = vbuf.at[vs, pl.ds(offs[p], pieces[p])]
        pltpu.make_async_copy(dst, dst, tailsem.at[p]).wait()
        acc = acc + lax.dot_general(lhs[:, offs[p]:offs[p] + pieces[p]],
                                    vbuf[vs, offs[p]:offs[p] + pieces[p], :],
                                    _NN, preferred_element_type=f32)
    out_ref[pl.ds(BH - 1, 1), :] = jnp.sum(acc, axis=0, keepdims=True) / d
    o_ref[...] = out_ref[...].astype(o_ref.dtype)


@jax.jit
def pallas_standalone__linear_kernel_rfa__decode_kernel(
    q: jax.Array,
    k: jax.Array,
    v: jax.Array,
    omega: jax.Array,
):
    B, H, S, D = k.shape
    M = omega.shape[0]
    BH = B * H
    assert q.shape == (B, H, 1, D) and M == 16 and D == 256 and S % _R == 0
    assert S // _R >= 2 and sum(_PIECES) == _R
    out = pl.pallas_call(
        _kernel,
        in_specs=[pl.BlockSpec(memory_space=pl.ANY)] * 4,
        out_specs=pl.BlockSpec(memory_space=pltpu.VMEM),
        out_shape=jax.ShapeDtypeStruct((BH, D), q.dtype),
        scratch_shapes=[
            pltpu.VMEM((_NB, _R, D), k.dtype),
            pltpu.VMEM((_NB - 1, _R, D), v.dtype),
            pltpu.VMEM((BH, D), q.dtype),
            pltpu.VMEM((M, D), omega.dtype),
            pltpu.SemaphoreType.DMA((_NB,)),
            pltpu.SemaphoreType.DMA((_NB - 1,)),
            pltpu.SemaphoreType.DMA((2,)),
            pltpu.SemaphoreType.DMA((len(_PIECES),)),
            pltpu.VMEM((BH, M, 128), jnp.float32),
            pltpu.VMEM((16, D), jnp.float32),
            pltpu.VMEM((8, 128), jnp.float32),
            pltpu.VMEM((BH, D), jnp.float32),
        ],
        compiler_params=pltpu.CompilerParams(
            vmem_limit_bytes=64 * 1024 * 1024,
            disable_bounds_checks=True,
            disable_semaphore_checks=True,
        ),
    )(q.reshape(BH, D), k.reshape(BH * S, D), v.reshape(BH * S, D), omega)
    return out.reshape(B, H, 1, D)
```

```python
import jax
import jax.numpy as jnp
from jax import lax
import jax.experimental.pallas as pl
import jax.experimental.pallas.tpu as pltpu

NT = (((1,), (1,)), ((), ()))
NN = (((1,), (0,)), ((), ()))

def make(R=2048, NB=4, bt=16, ns=4, sh=5, npieces=4, nobc=True, nosc=True):
    NBK, NBV = NB, NB - 1
    CT = R // 4
    W = CT // ns
    nblk = W // bt
    lg = ns.bit_length() - 1
    assert 1 << lg == ns and 0 <= sh < bt

    def kern(q_hbm, k_hbm, v_hbm, om_hbm, o_ref,
             kbuf, vbuf, qbuf, ombuf, ksem, vsem, auxsem,
             phiq_ref, acc_ref, den_ref, out_ref):
        BH, D = q_hbm.shape
        M = om_hbm.shape[0]
        TH = k_hbm.shape[0] // BH
        S = TH * 4
        CPH = S // R
        N = BH * CPH
        TS = TH // ns
        scale = float(D) ** -0.25
        inv_sqrt_m = float(M) ** -0.5
        f32 = jnp.float32
        bf16 = jnp.bfloat16

        def base_of(c):
            return (c // CPH) * TH + (c % CPH) * W

        def piece(src, base, dst, sem, t, o, n, prio):
            pltpu.make_async_copy(src.at[pl.ds(base + t * TS + o, n)],
                                  dst.at[pl.ds(t * W + o, n)], sem).start(priority=prio)

        def issue_pair(a, b):
            def go(nit, ofn, n):
                def f(s, _):
                    t = lax.bitwise_and(s, ns - 1)
                    u = lax.shift_right_logical(s, lg)
                    o = ofn(u)
                    piece(a[0], a[1], a[2], a[3], t, o, n, 0)
                    piece(b[0], b[1], b[2], b[3], t, o, n, 1)
                    return 0
                lax.fori_loop(0, nit, f, 0)
            if sh:
                go(ns, lambda u: 0, sh)
                go(ns * (nblk - 1), lambda u: sh + u * bt, bt)
                go(ns, lambda u: W - (bt - sh), bt - sh)
            else:
                go(ns * nblk, lambda u: u * bt, bt)

        def issue_single(a):
            hn = ns // 2
            def go(nit, ofn, n):
                def f(s, _):
                    t = lax.bitwise_and(s, hn - 1)
                    u = lax.shift_right_logical(s, lg - 1)
                    o = ofn(u)
                    piece(a[0], a[1], a[2], a[3], t, o, n, 0)
                    piece(a[0], a[1], a[2], a[3], t + hn, o, n, 1)
                    return 0
                lax.fori_loop(0, nit, f, 0)
            if sh:
                go(hn, lambda u: 0, sh)
                go(hn * (nblk - 1), lambda u: sh + u * bt, bt)
                go(hn, lambda u: W - (bt - sh), bt - sh)
            else:
                go(hn * nblk, lambda u: u * bt, bt)

        def kdesc(t):
            s_ = t % NBK
            return (k_hbm, base_of(t), kbuf.at[s_], ksem.at[s_])
        def vdesc(t):
            s_ = t % NBV
            return (v_hbm, base_of(t), vbuf.at[s_], vsem.at[s_])
        def k_wait(c):
            slot = c % NBK
            pltpu.make_async_copy(kbuf.at[slot], kbuf.at[slot], ksem.at[slot]).wait()
        def v_wait(c):
            slot = c % NBV
            pltpu.make_async_copy(vbuf.at[slot], vbuf.at[slot], vsem.at[slot]).wait()

        q_cp = pltpu.make_async_copy(q_hbm, qbuf, auxsem.at[0])
        om_cp = pltpu.make_async_copy(om_hbm, ombuf, auxsem.at[1])
        q_cp.start(); om_cp.start()
        issue_single(kdesc(0))
        for t in range(1, NB):
            issue_pair(kdesc(t), vdesc(t - 1))
        q_cp.wait(); om_cp.wait()

        om = ombuf[...]
        omf = om.astype(f32)
        qs_all = qbuf[...].astype(f32) * scale
        for h in range(BH):
            qs = qs_all[h:h + 1, :]
            t = omf * qs - 0.5 * (qs * qs)
            e = jnp.sum(t, axis=1, keepdims=True)
            phi_q = jnp.exp(e) * inv_sqrt_m + 1e-6
            phiq_ref[h] = jnp.broadcast_to(phi_q, (M, 128))
        ones = jnp.ones((M, D // 2), bf16)
        om_l = om[:, :128]
        om_r = om[:, 128:]

        def halves(x):
            nt = x.shape[0]
            x = x.reshape(nt // 2, 2, 8, 128)
            return x[:, 0].reshape(nt * 4, 128), x[:, 1].reshape(nt * 4, 128)

        def k_side(kt, phiq):
            kl, kr = halves(kt)
            n = kl.shape[0]
            pt = (lax.dot_general(om_l, kl, NT, preferred_element_type=f32)
                  + lax.dot_general(om_r, kr, NT, preferred_element_type=f32))
            klf = kl.astype(f32); krf = kr.astype(f32)
            sqp = (klf * klf + krf * krf).astype(bf16)
            kst = lax.dot_general(ones, sqp, NT, preferred_element_type=f32)
            e = pt * scale - kst * (0.5 * scale * scale)
            phi = jnp.exp(e) * inv_sqrt_m + 1e-6
            pw = phi * jnp.tile(phiq, (1, n // 128))
            w8 = pw[:8] + pw[8:]
            hi = w8.astype(bf16)
            lo = (w8 - hi.astype(f32)).astype(bf16)
            lhs = jnp.concatenate([hi, lo], axis=0)
            den = w8[:, 0:128]
            for t in range(1, n // 128):
                den = den + w8[:, t * 128:(t + 1) * 128]
            return lhs, den

        def v_side(lhs, vt):
            vl, vr = halves(vt)
            return jnp.concatenate([lax.dot_general(lhs, vl, NN, preferred_element_type=f32),
                                    lax.dot_general(lhs, vr, NN, preferred_element_type=f32)], axis=1)

        def total(den):
            return jnp.sum(jnp.sum(den, axis=0, keepdims=True), axis=1, keepdims=True) + 1e-6

        def body(c, carry):
            h = c // CPH
            j = c % CPH
            @pl.when(j == 0)
            def _():
                acc_ref[...] = jnp.zeros_like(acc_ref)
                den_ref[...] = jnp.zeros_like(den_ref)
            phiq = phiq_ref[h]
            k_wait(c)
            v_wait(c)
            lhs, dd = k_side(kbuf[c % NBK], phiq)
            acc = acc_ref[...] + v_side(lhs, vbuf[c % NBV])
            den = den_ref[...] + dd
            acc_ref[...] = acc
            den_ref[...] = den
            @pl.when(c + NB < N)
            def _():
                issue_pair(kdesc(c + NB), vdesc(c + NB - 1))
            @pl.when(c + NB == N)
            def _():
                issue_single(vdesc(N - 1))
            @pl.when(j == CPH - 1)
            def _():
                out_ref[pl.ds(h, 1), :] = jnp.sum(acc, axis=0, keepdims=True) / total(den)
            return carry

        lax.fori_loop(0, N - 1, body, 0)

        k_wait(N - 1)
        lhs, dd = k_side(kbuf[(N - 1) % NBK], phiq_ref[BH - 1])
        d = total(den_ref[...] + dd)
        v_wait(N - 1)
        acc = acc_ref[...] + v_side(lhs, vbuf[(N - 1) % NBV])
        out_ref[pl.ds(BH - 1, 1), :] = jnp.sum(acc, axis=0, keepdims=True) / d
        o_ref[...] = out_ref[...].astype(o_ref.dtype)

    def tiles(x):
        B, H, S, D = x.shape
        T = B * H * S
        return x.reshape(T // 8, 8, 2, 128).transpose(0, 2, 1, 3).reshape(T // 4, 8, 128)

    def f(q, k, v, om):
        B, H, S, D = k.shape
        M = om.shape[0]
        BH = B * H
        out = pl.pallas_call(
            kern,
            in_specs=[pl.BlockSpec(memory_space=pl.ANY)] * 4,
            out_specs=pl.BlockSpec(memory_space=pltpu.VMEM),
            out_shape=jax.ShapeDtypeStruct((BH, D), jnp.bfloat16),
            scratch_shapes=[
                pltpu.VMEM((NBK, CT, 8, 128), jnp.bfloat16), pltpu.VMEM((NBV, CT, 8, 128), jnp.bfloat16),
                pltpu.VMEM((BH, D), jnp.bfloat16), pltpu.VMEM((M, D), jnp.bfloat16),
                pltpu.SemaphoreType.DMA((NBK,)), pltpu.SemaphoreType.DMA((NBV,)),
                pltpu.SemaphoreType.DMA((2,)),
                pltpu.VMEM((BH, M, 128), jnp.float32),
                pltpu.VMEM((16, D), jnp.float32), pltpu.VMEM((8, 128), jnp.float32),
                pltpu.VMEM((BH, D), jnp.float32),
            ],
            compiler_params=pltpu.CompilerParams(vmem_limit_bytes=64 * 1024 * 1024,
                                                 disable_bounds_checks=nobc, disable_semaphore_checks=nosc),
        )(q.reshape(BH, D), tiles(k), tiles(v), om)
        return out.reshape(B, H, 1, D)
    return f


_SH = 5
_impl = make(sh=_SH)


@jax.jit
def pallas_standalone__linear_kernel_rfa__decode_kernel(q, k, v, omega):
    return _impl(q, k, v, omega)
```

```python
import jax
import jax.numpy as jnp
from jax import lax
import jax.experimental.pallas as pl
import jax.experimental.pallas.tpu as pltpu

_NT = (((1,), (1,)), ((), ()))
_NN = (((1,), (0,)), ((), ()))

_R = 2048
_NBUF = 4
_BT = 16
_NS = 4
_SH = 5
_PIECES = (4, 2, 2)

_CT = _R // 4
_W = _CT // _NS
_NBLK = _W // _BT


def _kernel(q_hbm, k_hbm, v_hbm, om_hbm, o_ref,
            buf, qbuf, ombuf, sem, auxsem, tailsem,
            phiq_ref, lhs_ref, acc_ref, den_ref, dent_ref, out_ref):
    NBUF, bt, ns, sh, pieces = _NBUF, _BT, _NS, _SH, _PIECES
    CT, W, nblk = _CT, _W, _NBLK
    lg = ns.bit_length() - 1
    P = len(pieces)
    poff = [sum(pieces[:p]) for p in range(P)]

    BH, D = q_hbm.shape
    M = om_hbm.shape[0]
    TH = k_hbm.shape[0] // BH
    CPH = TH // CT
    N = BH * CPH
    TS = TH // ns
    scale = float(D) ** -0.25
    inv_sqrt_m = float(M) ** -0.5
    f32 = jnp.float32
    bf16 = jnp.bfloat16

    def base_of(c):
        return (c // CPH) * TH + (c % CPH) * W

    def split(s):
        return lax.bitwise_and(s, ns - 1), lax.shift_right_logical(s, lg)

    def issue(slot, a, b):
        dst = buf.at[slot]
        sm = sem.at[slot]
        ab = base_of(a[1])
        bb = base_of(b[1])

        def cp(src, base, doff, t, o, n, prio):
            pltpu.make_async_copy(src.at[pl.ds(base + t * TS + o, n)],
                                  dst.at[pl.ds(doff + t * W + o, n)],
                                  sm).start(priority=prio)

        def cpb(src, base, doff, s, t, u, prio):
            pltpu.make_async_copy(src.at[pl.ds(base + t * TS + u * bt, bt)],
                                  dst.at[pl.ds(doff + s * bt, bt)],
                                  sm).start(priority=prio)

        def head(s, _):
            if not a[2]:
                cp(a[0], ab, 0, s, 0, sh, 0)
            cp(b[0], bb, CT, s, 0, sh, 1)
            return 0

        def mid(s, _):
            t, u = split(s)
            if a[2]:
                cpb(a[0], ab, 0, s, t, u, 0)
            else:
                cp(a[0], ab, 0, t, sh + u * bt, bt, 0)
            cp(b[0], bb, CT, t, sh + u * bt, bt, 1)
            return 0

        def tail(s, _):
            if a[2]:
                cpb(a[0], ab, 0, ns * (nblk - 1) + s, s, nblk - 1, 0)
            else:
                cp(a[0], ab, 0, s, W - (bt - sh), bt - sh, 0)
            cp(b[0], bb, CT, s, W - (bt - sh), bt - sh, 1)
            return 0

        lax.fori_loop(0, ns, head, 0)
        lax.fori_loop(0, ns * (nblk - 1), mid, 0)
        lax.fori_loop(0, ns, tail, 0)

    def issue_step(t):
        issue(t % NBUF, (k_hbm, t + 1, False), (v_hbm, t - 1, False))

    lslot = (N - 1) % NBUF

    def issue_last():
        dst = buf.at[lslot]
        ab = base_of(N - 2)
        bb = base_of(N - 1)

        def f(s, _):
            t, u = split(s)
            idx = 0
            t0 = 0
            nt = pieces[0] * ns * bt
            for p in range(1, P):
                ge = (u >= poff[p]).astype(jnp.int32)
                idx = idx + ge
                t0 = t0 + ge * (pieces[p - 1] * ns * bt)
                nt = nt + ge * ((pieces[p] - pieces[p - 1]) * ns * bt)
            sm = tailsem.at[idx]
            pltpu.make_async_copy(v_hbm.at[pl.ds(ab + t * TS + u * bt, bt)],
                                  dst.at[pl.ds(t0 + s * bt, bt)],
                                  sm).start(priority=0)
            pltpu.make_async_copy(v_hbm.at[pl.ds(bb + t * TS + u * bt, bt)],
                                  dst.at[pl.ds(t0 + nt + s * bt, bt)],
                                  sm).start(priority=1)
            return 0

        lax.fori_loop(0, ns * nblk, f, 0)

    def wait_slot(slot):
        pltpu.make_async_copy(buf.at[slot], buf.at[slot], sem.at[slot]).wait()

    q_cp = pltpu.make_async_copy(q_hbm, qbuf, auxsem.at[0])
    om_cp = pltpu.make_async_copy(om_hbm, ombuf, auxsem.at[1])
    q_cp.start()
    om_cp.start()
    issue(0, (k_hbm, 0, False), (k_hbm, 1, False))
    for t in range(1, NBUF):
        issue_step(t)
    q_cp.wait()
    om_cp.wait()

    om = ombuf[...]
    omf = om.astype(f32)
    qs_all = qbuf[...].astype(f32) * scale
    for h in range(BH):
        qs = qs_all[h:h + 1, :]
        e = jnp.sum(omf * qs - 0.5 * (qs * qs), axis=1, keepdims=True)
        phi_q = jnp.exp(e) * inv_sqrt_m + 1e-6
        phiq_ref[h] = jnp.broadcast_to(phi_q, (M, 128))
    ones = jnp.ones((M, 128), bf16)
    om_l = om[:, :128]
    om_r = om[:, 128:]

    def halves(x):
        nt = x.shape[0]
        x = x.reshape(nt // 2, 2, 8, 128)
        return x[:, 0].reshape(nt * 4, 128), x[:, 1].reshape(nt * 4, 128)

    def k_side(kt, phiq):
        kl, kr = halves(kt)
        n = kl.shape[0]
        pt = (lax.dot_general(om_l, kl, _NT, preferred_element_type=f32)
              + lax.dot_general(om_r, kr, _NT, preferred_element_type=f32))
        klf = kl.astype(f32)
        krf = kr.astype(f32)
        sqp = (klf * klf + krf * krf).astype(bf16)
        kst = lax.dot_general(ones, sqp, _NT, preferred_element_type=f32)
        e = pt * scale - kst * (0.5 * scale * scale)
        phi = jnp.exp(e) * inv_sqrt_m + 1e-6
        pw = phi * jnp.tile(phiq, (1, n // 128))
        w8 = pw[:8] + pw[8:]
        hi = w8.astype(bf16)
        lo = (w8 - hi.astype(f32)).astype(bf16)
        lhs = jnp.concatenate([hi, lo], axis=0)
        den = w8[:, 0:128]
        for t in range(1, n // 128):
            den = den + w8[:, t * 128:(t + 1) * 128]
        return lhs, den

    def v_side(lhs, vt):
        vl, vr = halves(vt)
        return jnp.concatenate(
            [lax.dot_general(lhs, vl, _NN, preferred_element_type=f32),
             lax.dot_general(lhs, vr, _NN, preferred_element_type=f32)], axis=1)

    def total(den):
        return jnp.sum(jnp.sum(den, axis=0, keepdims=True),
                       axis=1, keepdims=True) + 1e-6

    wait_slot(0)
    lhs0, dd0 = k_side(buf[0, 0:CT], phiq_ref[0])
    lhs_ref[0] = lhs0
    lhs1, dd1 = k_side(buf[0, CT:2 * CT], phiq_ref[0])
    lhs_ref[1] = lhs1
    den_ref[...] = dd0 + dd1
    acc_ref[...] = jnp.zeros_like(acc_ref)
    issue_step(NBUF)

    def body(t, carry):
        slot = t % NBUF
        ck = t + 1
        cv = t - 1
        hk = ck // CPH
        hv = cv // CPH
        vlast = (cv % CPH) == CPH - 1
        phiq = phiq_ref[hk]
        wait_slot(slot)
        lhs_n, dd = k_side(buf[slot, 0:CT], phiq)
        acc = acc_ref[...] + v_side(lhs_ref[cv % 3], buf[slot, CT:2 * CT])
        lhs_ref[ck % 3] = lhs_n
        den = jnp.where((ck % CPH) == 0, dd, den_ref[...] + dd)
        den_ref[...] = den
        tn = t + NBUF

        @pl.when(tn < N - 3)
        def _():
            issue_step(tn)

        @pl.when(tn == N - 3)
        def _():
            issue((N - 3) % NBUF, (k_hbm, N - 2, True), (v_hbm, N - 4, False))

        @pl.when(tn == N - 2)
        def _():
            issue((N - 2) % NBUF, (k_hbm, N - 1, True), (v_hbm, N - 3, False))

        @pl.when(tn == N - 1)
        def _():
            issue_last()

        @pl.when((ck % CPH) == CPH - 1)
        def _():
            dent_ref[hk] = den

        @pl.when(vlast)
        def _():
            out_ref[pl.ds(hv, 1), :] = (jnp.sum(acc, axis=0, keepdims=True)
                                        / total(dent_ref[hv]))
            acc_ref[...] = jnp.zeros_like(acc_ref)

        @pl.when(jnp.logical_not(vlast))
        def _():
            acc_ref[...] = acc

        return carry

    lax.fori_loop(1, N - 1, body, 0)

    d = total(den_ref[...])
    acc = acc_ref[...]
    for p in range(P):
        t0 = poff[p] * ns * bt
        nt = pieces[p] * ns * bt
        reg = buf.at[lslot, pl.ds(2 * t0, 2 * nt)]
        pltpu.make_async_copy(reg, reg, tailsem.at[p]).wait()
        acc = acc + v_side(lhs_ref[(N - 2) % 3, :, t0 * 4:(t0 + nt) * 4],
                           buf[lslot, 2 * t0:2 * t0 + nt])
        acc = acc + v_side(lhs_ref[(N - 1) % 3, :, t0 * 4:(t0 + nt) * 4],
                           buf[lslot, 2 * t0 + nt:2 * t0 + 2 * nt])
    out_ref[pl.ds(BH - 1, 1), :] = jnp.sum(acc, axis=0, keepdims=True) / d
    o_ref[...] = out_ref[...].astype(o_ref.dtype)


def _tiles(x):
    B, H, S, D = x.shape
    T = B * H * S
    return (x.reshape(T // 8, 8, 2, 128).transpose(0, 2, 1, 3)
            .reshape(T // 4, 8, 128))


@jax.jit
def pallas_standalone__linear_kernel_rfa__decode_kernel(
    q: jax.Array,
    k: jax.Array,
    v: jax.Array,
    omega: jax.Array,
):
    B, H, S, D = k.shape
    M = omega.shape[0]
    BH = B * H
    assert q.shape == (B, H, 1, D) and v.shape == k.shape
    assert D == 256 and M == 16 and S % _R == 0 and S // _R >= 3
    assert BH * (S // _R) >= _NBUF + 5
    assert sum(_PIECES) == _NBLK and 0 < _SH < _BT
    out = pl.pallas_call(
        _kernel,
        in_specs=[pl.BlockSpec(memory_space=pl.ANY)] * 4,
        out_specs=pl.BlockSpec(memory_space=pltpu.VMEM),
        out_shape=jax.ShapeDtypeStruct((BH, D), q.dtype),
        scratch_shapes=[
            pltpu.VMEM((_NBUF, 2 * _CT, 8, 128), k.dtype),
            pltpu.VMEM((BH, D), q.dtype),
            pltpu.VMEM((M, D), omega.dtype),
            pltpu.SemaphoreType.DMA((_NBUF,)),
            pltpu.SemaphoreType.DMA((2,)),
            pltpu.SemaphoreType.DMA((len(_PIECES),)),
            pltpu.VMEM((BH, M, 128), jnp.float32),
            pltpu.VMEM((3, 16, _R), jnp.bfloat16),
            pltpu.VMEM((16, D), jnp.float32),
            pltpu.VMEM((8, 128), jnp.float32),
            pltpu.VMEM((BH, 8, 128), jnp.float32),
            pltpu.VMEM((BH, D), jnp.float32),
        ],
        compiler_params=pltpu.CompilerParams(
            vmem_limit_bytes=64 * 1024 * 1024,
            disable_bounds_checks=True,
            disable_semaphore_checks=True,
        ),
    )(q.reshape(BH, D), _tiles(k), _tiles(v), omega)
    return out.reshape(B, H, 1, D)
```
